```python
import os as _os
_os.environ.setdefault("JAX_PLATFORMS", "cpu")
import jax
import jax.numpy as jnp

def _softmax(x, axis=-1):
    return jax.nn.softmax(x, axis=axis)
def _gelu(x):
    return jax.nn.gelu(x, approximate=True)
def _silu(x):
    return jax.nn.silu(x)
def _sigmoid(x):
    return jax.nn.sigmoid(x)
def _layernorm(x, axis=-1, eps=1e-5):
    m = jnp.mean(x, axis=axis, keepdims=True)
    v = jnp.var(x, axis=axis, keepdims=True)
    return (x - m) / jnp.sqrt(v + eps)
def _scatter_add(tgt, idx, src, axis=0):
    return tgt.at[idx].add(src)
def _segment_sum(src, seg, n):
    return jax.ops.segment_sum(src, seg, n)
class _Rng:
    def __init__(self, key):
        self._k = key
    def _next(self):
        self._k, sub = jax.random.split(self._k)
        return sub
    def normal(self, shape):
        return jax.random.normal(self._next(), shape, dtype=jnp.bfloat16)
    def randint(self, lo, hi, shape):
        return jax.random.randint(self._next(), shape, lo, hi, dtype=jnp.int32)
    def uniform(self, shape, lo=0.0, hi=1.0):
        return jax.random.uniform(self._next(), shape, jnp.bfloat16, lo, hi)
    def permutation(self, n):
        return jax.random.permutation(self._next(), n)


kernel_name = 'gated_mix__gqa_block_cached__dense_activation_squared_relu__decode'

def setup_inputs():
    _rng = _Rng(jax.random.key(int.from_bytes(__import__("os").urandom(4), "little")))
    _w = (lambda a: (lambda t: t.astype(jnp.bfloat16) if jnp.issubdtype(t.dtype, jnp.floating) else t)(jnp.asarray(a)))
    def _A_setup():
        B, Sq, D = 4, 1, 512
        Hq, Hkv, Sk, Dh = 32, 8, 4096, 128
        assert Hq % Hkv == 0, (Hq, Hkv)
        return {
            "x": _w((lambda *s: _rng.normal(s) * 0.05)(B, Sq, D)),
            "k_cache": _w((lambda *s: _rng.normal(s) * 3.2)(B, Hkv, Sk, Dh)),
            "v_cache": _w((lambda *s: _rng.normal(s) * 1.6)(B, Hkv, Sk, Dh)),
            "wq": _w((lambda *s: _rng.normal(s) * 3.2)(D, Hq * Dh) * (D ** -0.5)),
            "wo": _w((lambda *s: _rng.normal(s) * 1.6)(Hq * Dh, D) * ((Hq * Dh) ** -0.5)),
        }
    _A_in = _A_setup()

    def _B_setup():
        B, S, D, F = 4, 1, 512, 1792
        return {
            "x": _w((lambda *s: _rng.normal(s) * 0.05)(B, S, D)),
            "w1": _w((lambda *s: _rng.normal(s) * 0.1)(D, F)),
            "b1": _w((lambda *s: _rng.normal(s) * 0.05)(F)),
            "w2": _w((lambda *s: _rng.normal(s) * 0.05)(F, D)),
            "b2": _w((lambda *s: _rng.normal(s) * 0.05)(D)),
        }
    _B_in = _B_setup()

    return {
        "A_x": _A_in["x"],
        "A_k_cache": _A_in["k_cache"],
        "A_v_cache": _A_in["v_cache"],
        "A_wq": _A_in["wq"],
        "A_wo": _A_in["wo"],
        "B_x": _B_in["x"],
        "B_w1": _B_in["w1"],
        "B_b1": _B_in["b1"],
        "B_w2": _B_in["w2"],
        "B_b2": _B_in["b2"],
        "gate_w": _w((lambda *s: _rng.normal(s) * 0.05)(512) * 16.0),
    }

def reference(A_x, A_k_cache, A_v_cache, A_wq, A_wo, B_x, B_w1, B_b1, B_w2, B_b2, gate_w):
    def _A_ref(x, k_cache, v_cache, wq, wo):
        B, Sq, D = x.shape
        Hq, Dh = 32, 128
        Hkv = k_cache.shape[1]
        rep = Hq // Hkv
        q = (lambda x, *d: x.transpose(*d))((x @ wq).reshape(B, Sq, Hq, Dh), 0, 2, 1, 3)
        k = jnp.repeat(k_cache, rep, axis=1)
        v = jnp.repeat(v_cache, rep, axis=1)
        scores = jnp.einsum("bhqd,bhkd->bhqk", q, k) * (Dh ** -0.5)
        p = _softmax(scores, axis=-1)
        o = jnp.einsum("bhqk,bhkd->bhqd", p, v)
        return (lambda x, *d: x.transpose(*d))(o, 0, 2, 1, 3).reshape(B, Sq, Hq * Dh) @ wo

    def _B_ref(x, w1, b1, w2, b2):
        h = jnp.einsum("bsd,df->bsf", x, w1) + b1
        zero = jnp.zeros_like(h)
        r = jnp.where(h > zero, h, zero)
        h = r * r
        out = jnp.einsum("bsf,fd->bsd", h, w2) + b2
        return out

    x = A_x
    g = _sigmoid((x * gate_w).sum(-1, keepdims=True))
    a = _A_ref(x, A_k_cache, A_v_cache, A_wq, A_wo)
    b = _B_ref(x, B_w1, B_b1, B_w2, B_b2)
    return g * a + (1 - g) * b
```

```python
import functools

import jax
import jax.numpy as jnp
import jax.experimental.pallas as pl
import jax.experimental.pallas.tpu as pltpu


def _kernel(x_hbm, k_hbm, v_hbm, wq_hbm, wo_hbm, w1_hbm, b1_hbm, w2_hbm, b2_hbm,
            gw_hbm, out_ref,
            x_v, wq_v, wo_v, w1_v, w2_v, b1_v, b2_v, gw_v, kbuf, vbuf,
            qs, osc, acc, ffn, sem_s, sem_w, sem_k, sem_v,
            *, B, D, HKV, G, DH, scale):
    f32 = jnp.float32
    bf16 = jnp.bfloat16
    NBUF = B

    small_copies = [
        pltpu.make_async_copy(x_hbm, x_v, sem_s.at[0]),
        pltpu.make_async_copy(gw_hbm, gw_v, sem_s.at[1]),
        pltpu.make_async_copy(b1_hbm, b1_v, sem_s.at[2]),
        pltpu.make_async_copy(b2_hbm, b2_v, sem_s.at[3]),
    ]
    wq_copy = pltpu.make_async_copy(wq_hbm, wq_v, sem_w.at[0])
    w1_copy = pltpu.make_async_copy(w1_hbm, w1_v, sem_w.at[1])
    w2_copy = pltpu.make_async_copy(w2_hbm, w2_v, sem_w.at[2])
    wo_copy = pltpu.make_async_copy(wo_hbm, wo_v, sem_w.at[3])

    def k_copy(h, b):
        return pltpu.make_async_copy(k_hbm.at[b, h], kbuf.at[b], sem_k.at[b])

    def v_copy(h, b):
        return pltpu.make_async_copy(v_hbm.at[b, h], vbuf.at[b], sem_v.at[b])

    for c in small_copies:
        c.start()
    wq_copy.start()
    for b in range(NBUF - 1):
        k_copy(0, b).start()
        v_copy(0, b).start()

    for c in small_copies:
        c.wait()
    x = x_v[0]

    rows = jax.lax.broadcasted_iota(jnp.int32, (B * G, B), 0)
    cols = jax.lax.broadcasted_iota(jnp.int32, (B * G, B), 1)
    sel = (rows // G == cols).astype(bf16)
    x16 = jnp.dot(sel, x, preferred_element_type=f32).astype(bf16)

    wq_copy.wait()
    rowg = jax.lax.broadcasted_iota(jnp.int32, (B * G, DH), 0) % G
    for h in range(HKV):
        qfull = jnp.dot(x16, wq_v[:, h * G * DH:(h + 1) * G * DH],
                        preferred_element_type=f32)
        qh = jnp.zeros((B * G, DH), f32)
        for g in range(G):
            qh = jnp.where(rowg == g, qfull[:, g * DH:(g + 1) * DH], qh)
        qs[h] = qh

    acc[...] = jnp.zeros(acc.shape, f32)

    def body(h, carry):
        for b in range(B):
            nb = (b + NBUF - 1) % B
            dh_ = (b + NBUF - 1) // B

            @pl.when(h + dh_ < HKV)
            def _():
                k_copy(h + dh_, nb).start()
                v_copy(h + dh_, nb).start()

            if b == 1:
                @pl.when(h == 0)
                def _():
                    wo_copy.start()

                @pl.when(h == 1)
                def _():
                    w1_copy.start()

                @pl.when(h == 2)
                def _():
                    w2_copy.start()

            k_copy(h, b).wait()
            q = qs[h, pl.ds(b * G, G), :].astype(bf16)
            s = jax.lax.dot_general(q, kbuf[b], (((1,), (1,)), ((), ())),
                                    preferred_element_type=f32)
            s = s * scale
            m = jnp.max(s, axis=-1, keepdims=True)
            p = jnp.exp(s - m)
            l = jnp.sum(p, axis=-1, keepdims=True)
            v_copy(h, b).wait()
            o = jnp.dot(p.astype(bf16), vbuf[b], preferred_element_type=f32)
            osc[pl.ds(b * G, G), :] = o / l

        @pl.when(h == 4)
        def _():
            w1_copy.wait()
            hid = jnp.dot(x, w1_v[...], preferred_element_type=f32) + b1_v[...].astype(f32).reshape(1, -1)
            r = jnp.maximum(hid, 0.0)
            hid = (r * r).astype(bf16)
            w2_copy.wait()
            ffn[...] = jnp.dot(hid, w2_v[...], preferred_element_type=f32) + b2_v[...].astype(f32).reshape(1, -1)

        @pl.when(h == 0)
        def _():
            wo_copy.wait()

        _wo_proj(h)

        return carry

    def _wo_proj(h):
        a = acc[...]
        for g in range(G):
            og = osc[pl.ds(g, B, stride=G), :].astype(bf16)
            start = pl.multiple_of((h * G + g) * DH, DH)
            a = a + jnp.dot(og, wo_v[pl.ds(start, DH), :], preferred_element_type=f32)
        acc[...] = a

    jax.lax.fori_loop(0, HKV, body, 0)

    xf = x.astype(f32)
    gate = jax.nn.sigmoid(jnp.sum(xf * gw_v[...].astype(f32).reshape(1, -1), axis=-1, keepdims=True))
    out_ref[0] = (gate * acc[...] + (1.0 - gate) * ffn[...]).astype(out_ref.dtype)


@jax.jit
def pallas_gated_mix__gqa_block_cached__dense_activation_squared_relu__decode_kernel(
    A_x: jax.Array,
    A_k_cache: jax.Array,
    A_v_cache: jax.Array,
    A_wq: jax.Array,
    A_wo: jax.Array,
    B_x: jax.Array,
    B_w1: jax.Array,
    B_b1: jax.Array,
    B_w2: jax.Array,
    B_b2: jax.Array,
    gate_w: jax.Array,
):
    del B_x
    B, SQ, D = A_x.shape
    assert SQ == 1
    _, HKV, SK, DH = A_k_cache.shape
    HQ = A_wq.shape[1] // DH
    G = HQ // HKV
    F = B_w1.shape[1]
    scale = float(DH) ** -0.5
    assert HKV > 4 and B >= 2

    any_spec = pl.BlockSpec(memory_space=pl.ANY)
    bf16 = jnp.bfloat16
    f32 = jnp.float32
    scratch = [
        pltpu.VMEM((SQ, B, D), bf16),
        pltpu.VMEM((D, HQ * DH), bf16),
        pltpu.VMEM((HQ * DH, D), bf16),
        pltpu.VMEM((D, F), bf16),
        pltpu.VMEM((F, D), bf16),
        pltpu.VMEM((F,), bf16),
        pltpu.VMEM((D,), bf16),
        pltpu.VMEM((D,), bf16),
        pltpu.VMEM((B, SK, DH), bf16),
        pltpu.VMEM((B, SK, DH), bf16),
        pltpu.VMEM((HKV, B * G, DH), f32),
        pltpu.VMEM((B * G, DH), f32),
        pltpu.VMEM((B, D), f32),
        pltpu.VMEM((B, D), f32),
        pltpu.SemaphoreType.DMA((4,)),
        pltpu.SemaphoreType.DMA((4,)),
        pltpu.SemaphoreType.DMA((B,)),
        pltpu.SemaphoreType.DMA((B,)),
    ]
    out = pl.pallas_call(
        functools.partial(_kernel, B=B, D=D, HKV=HKV, G=G, DH=DH, scale=scale),
        out_shape=jax.ShapeDtypeStruct((SQ, B, D), A_x.dtype),
        in_specs=[any_spec] * 10,
        out_specs=pl.BlockSpec(memory_space=pltpu.VMEM),
        scratch_shapes=scratch,
        compiler_params=pltpu.CompilerParams(vmem_limit_bytes=64 * 1024 * 1024),
    )(A_x.transpose(1, 0, 2), A_k_cache, A_v_cache, A_wq, A_wo, B_w1, B_b1, B_w2, B_b2, gate_w)
    return out.transpose(1, 0, 2)
```
